```python
import os as _os
_os.environ.setdefault("JAX_PLATFORMS", "cpu")
import jax
import jax.numpy as jnp

def _softmax(x, axis=-1):
    return jax.nn.softmax(x, axis=axis)
def _gelu(x):
    return jax.nn.gelu(x, approximate=True)
def _silu(x):
    return jax.nn.silu(x)
def _sigmoid(x):
    return jax.nn.sigmoid(x)
def _layernorm(x, axis=-1, eps=1e-5):
    m = jnp.mean(x, axis=axis, keepdims=True)
    v = jnp.var(x, axis=axis, keepdims=True)
    return (x - m) / jnp.sqrt(v + eps)
def _scatter_add(tgt, idx, src, axis=0):
    return tgt.at[idx].add(src)
def _segment_sum(src, seg, n):
    return jax.ops.segment_sum(src, seg, n)
class _Rng:
    def __init__(self, key):
        self._k = key
    def _next(self):
        self._k, sub = jax.random.split(self._k)
        return sub
    def normal(self, shape):
        return jax.random.normal(self._next(), shape, dtype=jnp.bfloat16)
    def randint(self, lo, hi, shape):
        return jax.random.randint(self._next(), shape, lo, hi, dtype=jnp.int32)
    def uniform(self, shape, lo=0.0, hi=1.0):
        return jax.random.uniform(self._next(), shape, jnp.bfloat16, lo, hi)
    def permutation(self, n):
        return jax.random.permutation(self._next(), n)


kernel_name = 'sequential_preLN__compressed_kv_cla__dense_activation_mish__decode'

def setup_inputs():
    _rng = _Rng(jax.random.key(int.from_bytes(__import__("os").urandom(4), "little")))
    _w = (lambda a: (lambda t: t.astype(jnp.bfloat16) if jnp.issubdtype(t.dtype, jnp.floating) else t)(jnp.asarray(a)))
    def _A_setup():
        B, H, Sq, Sk, D, M = 2, 32, 1, 8192, 128, 512
        Dc = 4 * D
        return {
            "x": _w((lambda *s: _rng.normal(s) * 0.05)(B, Sq, M)),
            "c_kv": _w((lambda *s: _rng.normal(s) * 0.8)(B, Sk, Dc)),
            "w_q": _w((lambda *s: _rng.normal(s) * 0.8)(M, H, D) * (M ** -0.5)),
            "w_uk": _w((lambda *s: _rng.normal(s) * 0.8)(Dc, H, D) * (Dc ** -0.5)),
            "w_uv": _w((lambda *s: _rng.normal(s) * 0.8)(Dc, H, D) * (Dc ** -0.5)),
            "w_o": _w((lambda *s: _rng.normal(s) * 0.8)(H, D, M) * ((H * D) ** -0.5)),
        }
    _A_in = _A_setup()

    def _B_setup():
        B, S, D, F = 2, 1, 512, 1792
        return {
            "x": _w((lambda *s: _rng.normal(s) * 0.05)(B, S, D)),
            "w1": _w((lambda *s: _rng.normal(s) * 0.4)(D, F) * (D ** -0.5)),
            "b1": _w((lambda *s: _rng.normal(s) * 0.05)(F)),
            "w2": _w((lambda *s: _rng.normal(s) * 0.05)(F, D) * (F ** -0.5)),
        }
    _B_in = _B_setup()

    return {
        "A_x": _A_in["x"],
        "A_c_kv": _A_in["c_kv"],
        "A_w_q": _A_in["w_q"],
        "A_w_uk": _A_in["w_uk"],
        "A_w_uv": _A_in["w_uv"],
        "A_w_o": _A_in["w_o"],
        "B_x": _B_in["x"],
        "B_w1": _B_in["w1"],
        "B_b1": _B_in["b1"],
        "B_w2": _B_in["w2"],
    }

def reference(A_x, A_c_kv, A_w_q, A_w_uk, A_w_uv, A_w_o, B_x, B_w1, B_b1, B_w2):
    def _A_ref(x, c_kv, w_q, w_uk, w_uv, w_o):
        B, Sq, M = x.shape[0], x.shape[1], x.shape[2]
        Sk = c_kv.shape[1]
        H, D = w_q.shape[1], w_q.shape[2]
        q = jnp.einsum("bqm,mhd->bhqd", x, w_q)
        k = jnp.einsum("bkc,chd->bhkd", c_kv, w_uk)
        v = jnp.einsum("bkc,chd->bhkd", c_kv, w_uv)
        scores = jnp.einsum("bhqd,bhkd->bhqk", q, k) * (D ** -0.5)
        off = Sk - Sq
        qi = jnp.arange(Sq)[:, None]
        kj = jnp.arange(Sk)[None, :]
        cmask = kj <= (qi + off)
        scores = jnp.where(cmask[None, None], scores, -1e9)
        p = _softmax(scores, axis=-1)
        ctx = jnp.einsum("bhqk,bhkd->bhqd", p, v)
        return jnp.einsum("bhqd,hdm->bqm", ctx, w_o)

    def _B_ref(x, w1, b1, w2):
        h = jnp.einsum("bsd,df->bsf", x, w1) + b1
        sp = jnp.log1p(jnp.exp(-jnp.abs(h))) + jnp.where(h > 0, h, jnp.zeros_like(h))
        act = h * jnp.tanh(sp)
        return jnp.einsum("bsf,fd->bsd", act, w2)

    x = A_x
    h = x + _A_ref(_layernorm(x, axis=-1), A_c_kv, A_w_q, A_w_uk, A_w_uv, A_w_o)
    h2 = h + _B_ref(_layernorm(h, axis=-1), B_w1, B_b1, B_w2)
    return h2
```

```python
import jax
import jax.numpy as jnp
from jax import lax
from jax.experimental import pallas as pl
from jax.experimental.pallas import tpu as pltpu

F32 = jnp.float32
BF16 = jnp.bfloat16

_B, _H, _D, _M, _DC, _SK, _F = 2, 32, 128, 512, 512, 8192, 1792
_EPS = 1e-5
_LOG2E = 1.4426950408889634

_CK = 1024
_DEPTH = 3
_WROWS = 128
_OHEADS = 8
_W1_ROWS = (256, 256)
_W2_ROWS = (512, 512, 384, 256, 128)


def _layernorm(x):
    m = jnp.mean(x, axis=-1, keepdims=True)
    d = x - m
    v = jnp.mean(d * d, axis=-1, keepdims=True)
    return d * lax.rsqrt(v + _EPS)


def _dot(a, b):
    return jnp.dot(a, b, preferred_element_type=F32)


def _dot_nt(a, b):
    return lax.dot_general(a, b, (((1,), (1,)), ((), ())), preferred_element_type=F32)


def _kernel(x_ref, b1_ref, ckv_hbm, wq_hbm, wuk_hbm, wuv_hbm, wo_hbm, w1_hbm, w2_hbm,
            o_ref,
            ckv_s, wq_s, wuk_s, wuv_s, wo_s, w1_s, w2_s, y_s, qa_s, cc_s, sems):
    plan = []

    def add(src, dst):
        plan.append((src, dst))
        return len(plan) - 1

    def add_rows(hbm, vmem, sizes):
        ids, s = [], 0
        for n in sizes:
            ids.append(add(hbm.at[pl.ds(s, n)], vmem.at[pl.ds(s, n)]))
            s += n
        return ids

    nw = _M // _WROWS
    ids_q = add_rows(wq_hbm, wq_s, [_WROWS] * nw)
    ids_uk = add_rows(wuk_hbm, wuk_s, [_WROWS] * nw)
    nck = _SK // _CK
    ids_kv = [add(ckv_hbm.at[b, pl.ds(c * _CK, _CK)], ckv_s.at[b, pl.ds(c * _CK, _CK)])
              for b in range(_B) for c in range(nck)]
    ids_uv = add_rows(wuv_hbm, wuv_s, [_WROWS] * nw)
    ids_o = add_rows(wo_hbm, wo_s, [_OHEADS] * (_H // _OHEADS))
    ids_1 = add_rows(w1_hbm, w1_s, list(_W1_ROWS))
    ids_2 = add_rows(w2_hbm, w2_s, list(_W2_ROWS))
    n_copies = len(plan)

    def copy(i):
        return pltpu.make_async_copy(plan[i][0], plan[i][1], sems.at[i % _DEPTH])

    def arrive(i):
        copy(i).wait()
        if i + _DEPTH < n_copies:
            copy(i + _DEPTH).start()

    for i in range(_DEPTH):
        copy(i).start()

    row = lax.broadcasted_iota(jnp.int32, (32, 128), 0)
    lane = lax.broadcasted_iota(jnp.int32, (32, 128), 1)
    hl = row % 16
    diag = (lane % 16) == hl

    x = x_ref[...].astype(F32)
    xn = _layernorm(x).astype(BF16).astype(F32)
    for i in range(4):
        y_s[0, 2 * i:2 * i + 2, :] = xn[:, 128 * i:128 * (i + 1)]
    x8 = y_s[0]
    lane8 = lax.broadcasted_iota(jnp.int32, (8, 128), 1)
    for t in range(16):
        y_s[t] = jnp.take_along_axis(x8, 8 * t + lane8 // 16, axis=1)

    nt = _WROWS // 8
    q = [jnp.zeros((32, 128), F32) for _ in range(2)]
    for ci, cid in enumerate(ids_q):
        lhs = []
        for t in range(nt):
            g = ci * nt + t
            i, tt = g // 16, g % 16
            rows = [jnp.broadcast_to(y_s[tt, 2 * i + b:2 * i + b + 1, :], (16, 128)) for b in range(2)]
            lhs.append(jnp.where(diag, jnp.concatenate(rows, axis=0), 0.0).astype(BF16))
        lhs = jnp.concatenate(lhs, axis=1)
        arrive(cid)
        for j in range(2):
            w = wq_s[ci * _WROWS:(ci + 1) * _WROWS, 16 * j:16 * j + 16, :].reshape(16 * _WROWS, 128)
            q[j] = q[j] + _dot(lhs, w)
    qb = [t.astype(BF16) for t in q]

    idx_c = (lane % 8) * 16 + hl
    for ci, cid in enumerate(ids_uk):
        arrive(cid)
        for j in range(2):
            for blk in range(_WROWS // 128):
                out = jnp.zeros((32, 128), F32)
                for sub in range(4):
                    c0 = ci * _WROWS + blk * 128 + sub * 32
                    w = wuk_s[c0:c0 + 32, 16 * j:16 * j + 16, :].reshape(512, 128)
                    s = _dot_nt(qb[j], w)
                    for u in range(4):
                        g = jnp.take_along_axis(s[:, 128 * u:128 * (u + 1)], idx_c, axis=1)
                        out = jnp.where(lane // 8 == sub * 4 + u, g, out)
                c0 = ci * _WROWS + blk * 128
                ob = out.astype(BF16)
                for b in range(2):
                    qa_s[b, 16 * j:16 * j + 16, c0:c0 + 128] = ob[16 * b:16 * b + 16, :]

    cexp = (_D ** -0.5) * _LOG2E
    for b in range(_B):
        qa = qa_s[b]
        m = jnp.full((32, 1), -jnp.inf, F32)
        l = jnp.zeros((32, 128), F32)
        acc = jnp.zeros((32, _DC), F32)
        for c in range(nck):
            arrive(ids_kv[b * nck + c])
            kv = ckv_s[b, c * _CK:(c + 1) * _CK, :]
            s = _dot_nt(qa, kv)
            m_new = jnp.maximum(m, jnp.max(s, axis=1, keepdims=True))
            alpha = jnp.exp2((m - m_new) * cexp)
            p = jnp.exp2((s - m_new) * cexp)
            ps = p[:, 0:128]
            for u in range(1, _CK // 128):
                ps = ps + p[:, 128 * u:128 * (u + 1)]
            l = l * alpha + ps
            acc = acc * alpha + _dot(p.astype(BF16), kv)
            m = m_new
        cc = acc / jnp.sum(l, axis=1, keepdims=True)
        for j in range(2):
            cc_s[j, 16 * b:16 * b + 16, :] = cc[16 * j:16 * j + 16, :]

    ctx = [jnp.zeros((32, 128), F32) for _ in range(2)]
    for ci, cid in enumerate(ids_uv):
        lhs = []
        for j in range(2):
            parts = []
            for t in range(nt):
                g = ci * nt + t
                i, tt = g // 16, g % 16
                z = jnp.take_along_axis(cc_s[j, :, 128 * i:128 * (i + 1)], 8 * tt + lane // 16, axis=1)
                parts.append(jnp.where(diag, z, 0.0).astype(BF16))
            lhs.append(jnp.concatenate(parts, axis=1))
        arrive(cid)
        for j in range(2):
            w = wuv_s[ci * _WROWS:(ci + 1) * _WROWS, 16 * j:16 * j + 16, :].reshape(16 * _WROWS, 128)
            ctx[j] = ctx[j] + _dot(lhs[j], w)

    oacc = jnp.zeros((32, _M), F32)
    for ci, cid in enumerate(ids_o):
        parts = []
        for k in range(_OHEADS):
            h = ci * _OHEADS + k
            parts.append(jnp.where(hl == h % 16, ctx[h // 16], 0.0).astype(BF16))
        lhs = jnp.concatenate(parts, axis=1)
        arrive(cid)
        w = wo_s[ci * _OHEADS:(ci + 1) * _OHEADS].reshape(128 * _OHEADS, _M)
        oacc = oacc + _dot(lhs, w)
    o0 = jnp.sum(oacc[0:16], axis=0, keepdims=True)
    o1 = jnp.sum(oacc[16:32], axis=0, keepdims=True)
    r2 = lax.broadcasted_iota(jnp.int32, (2, _M), 0)
    attn = jnp.where(r2 == 0, jnp.broadcast_to(o0, (2, _M)), jnp.broadcast_to(o1, (2, _M)))
    h = x + attn

    hn = _layernorm(h).astype(BF16)
    h1 = jnp.broadcast_to(b1_ref[...].astype(F32).reshape(1, _F), (2, _F))
    s = 0
    for cid, n in zip(ids_1, _W1_ROWS):
        arrive(cid)
        h1 = h1 + _dot(hn[:, s:s + n], w1_s[s:s + n, :])
        s += n
    sp = jnp.log1p(jnp.exp(-jnp.abs(h1))) + jnp.maximum(h1, 0.0)
    act = (h1 * jnp.tanh(sp)).astype(BF16)
    out = h
    s = 0
    for cid, n in zip(ids_2, _W2_ROWS):
        arrive(cid)
        out = out + _dot(act[:, s:s + n], w2_s[s:s + n, :])
        s += n
    o_ref[...] = out.astype(o_ref.dtype)


@jax.jit
def pallas_sequential_preLN__compressed_kv_cla__dense_activation_mish__decode_kernel(
    A_x: jax.Array,
    A_c_kv: jax.Array,
    A_w_q: jax.Array,
    A_w_uk: jax.Array,
    A_w_uv: jax.Array,
    A_w_o: jax.Array,
    B_x: jax.Array,
    B_w1: jax.Array,
    B_b1: jax.Array,
    B_w2: jax.Array,
):
    del B_x
    b, sq, m = A_x.shape
    hbm = pl.BlockSpec(memory_space=pl.ANY)
    out = pl.pallas_call(
        _kernel,
        out_shape=jax.ShapeDtypeStruct((b * sq, m), A_x.dtype),
        in_specs=[pl.BlockSpec(memory_space=pltpu.VMEM), pl.BlockSpec(memory_space=pltpu.VMEM)] + [hbm] * 7,
        out_specs=pl.BlockSpec(memory_space=pltpu.VMEM),
        scratch_shapes=[
            pltpu.VMEM(A_c_kv.shape, A_c_kv.dtype),
            pltpu.VMEM(A_w_q.shape, A_w_q.dtype),
            pltpu.VMEM(A_w_uk.shape, A_w_uk.dtype),
            pltpu.VMEM(A_w_uv.shape, A_w_uv.dtype),
            pltpu.VMEM(A_w_o.shape, A_w_o.dtype),
            pltpu.VMEM(B_w1.shape, B_w1.dtype),
            pltpu.VMEM(B_w2.shape, B_w2.dtype),
            pltpu.VMEM((16, 8, 128), F32),
            pltpu.VMEM((_B, _H, _DC), BF16),
            pltpu.VMEM((2, 32, _DC), F32),
            pltpu.SemaphoreType.DMA((_DEPTH,)),
        ],
        compiler_params=pltpu.CompilerParams(vmem_limit_bytes=100 * 1024 * 1024),
    )(A_x.reshape(b * sq, m), B_b1, A_c_kv, A_w_q, A_w_uk, A_w_uv, A_w_o, B_w1, B_w2)
    return out.reshape(b, sq, m)
```

```python
import jax
import jax.numpy as jnp
from jax import lax
from jax.experimental import pallas as pl
from jax.experimental.pallas import tpu as pltpu

F32 = jnp.float32
BF16 = jnp.bfloat16

_B, _H, _D, _M, _DC, _SK, _F = 2, 32, 128, 512, 512, 8192, 1792
_EPS = 1e-5
_LOG2E = 1.4426950408889634

_RING = 6
_NSW = 8
_GW = 8
_NSK = 16
_GK = 16
_NSO = 8
_GO = 8
_F_STEPS = (256,) * 7
_LEAD = 1
_CKG = 2


def _layernorm(x):
    m = jnp.mean(x, axis=-1, keepdims=True)
    d = x - m
    v = jnp.mean(d * d, axis=-1, keepdims=True)
    return d * lax.rsqrt(v + _EPS)


def _dot(a, b):
    return jnp.dot(a, b, preferred_element_type=F32)


def _dot_nt(a, b):
    return lax.dot_general(a, b, (((1,), (1,)), ((), ())), preferred_element_type=F32)


def _kernel(x_hbm, b1_hbm, ckv_hbm, wq_hbm, wuk_hbm, wuv_hbm, wo_hbm, w1_hbm, w2_hbm,
            o_ref,
            ckv_s, wq_s, wuk_s, wuv_s, wo_s, w1_s, w2_s, y_s, qa_s, cc_s, x_s, b1_s, sems):
    groups = []

    def add_group(copies, slab):
        groups.append((copies, slab))
        return len(groups) - 1

    def add_weight(hbm, vmem):
        return [add_group([(hbm.at[s, g, pl.ds(r, 4)], vmem.at[s, g, pl.ds(r, 4)])
                           for r in (0, 4) for s in range(_NSW)], vmem.at[:, g])
                for g in range(_GW)]

    g_small = add_group([(x_hbm, x_s), (b1_hbm, b1_s)], None)
    g_q = add_weight(wq_hbm, wq_s)
    g_uk = add_weight(wuk_hbm, wuk_s)
    g_kv = [[add_group([(ckv_hbm.at[b, s, c], ckv_s.at[b, s, c]) for s in range(_NSK)], ckv_s.at[b, :, c])
             for c in range(_GK)] for b in range(_B)]
    g_uv = add_weight(wuv_hbm, wuv_s)
    g_o = [add_group([(wo_hbm.at[s, g, pl.ds(r, 32)], wo_s.at[s, g, pl.ds(r, 32)])
                      for r in (0, 32) for s in range(_NSO)], wo_s.at[:, g])
           for g in range(_GO)]
    nf = len(_F_STEPS)
    f_lo = [sum(_F_STEPS[:f]) for f in range(nf)]
    g_1, g_2 = [None] * nf, [None] * nf

    def add_w1(f):
        cols = pl.ds(f_lo[f], _F_STEPS[f])
        rows = 16384 // _F_STEPS[f]
        g_1[f] = add_group([(w1_hbm.at[pl.ds(r, rows), cols], w1_s.at[pl.ds(r, rows), cols])
                            for r in range(0, _M, rows)], w1_s.at[:, cols])

    def add_w2(f):
        g_2[f] = add_group([(w2_hbm.at[pl.ds(f_lo[f] + r, 32)], w2_s.at[pl.ds(f_lo[f] + r, 32)])
                            for r in range(0, _F_STEPS[f], 32)], w2_s.at[pl.ds(f_lo[f], _F_STEPS[f])])

    for f in range(nf + _LEAD - 1):
        if f < nf:
            add_w1(f)
        if f >= _LEAD - 1:
            add_w2(f - _LEAD + 1)
    n_groups = len(groups)
    issued = [0]

    def start(g):
        for src, dst in groups[g][0]:
            pltpu.make_async_copy(src, dst, sems.at[g % _RING]).start(priority=issued[0] % 2)
            issued[0] += 1

    def arrive(g):
        copies, slab = groups[g]
        if slab is None:
            for src, dst in copies:
                pltpu.make_async_copy(src, dst, sems.at[g % _RING]).wait()
        else:
            pltpu.make_async_copy(slab, slab, sems.at[g % _RING]).wait()
        if g + _RING < n_groups:
            start(g + _RING)

    for g in range(_RING):
        start(g)

    row = lax.broadcasted_iota(jnp.int32, (32, 128), 0)
    lane = lax.broadcasted_iota(jnp.int32, (32, 128), 1)
    hl = row % 16
    diag = (lane % 16) == hl

    arrive(g_small)
    x = x_s[...].astype(F32)
    xn = _layernorm(x).astype(BF16).astype(F32)
    for i in range(4):
        y_s[0, 2 * i:2 * i + 2, :] = xn[:, 128 * i:128 * (i + 1)]
    x8 = y_s[0]
    lane8 = lax.broadcasted_iota(jnp.int32, (8, 128), 1)
    for t in range(16):
        y_s[t] = jnp.take_along_axis(x8, 8 * t + lane8 // 16, axis=1)

    def tile_pos(s, g):
        return s // 2, 8 * (s % 2) + g

    def w_tile(ref, g, j):
        return ref[:, g, :, 16 * j:16 * j + 16, :].reshape(_NSW * 128, 128)

    q = [jnp.zeros((32, 128), F32) for _ in range(2)]
    for g in range(_GW):
        lhs = []
        for s in range(_NSW):
            i, t = tile_pos(s, g)
            rows = [jnp.broadcast_to(y_s[t, 2 * i + b:2 * i + b + 1, :], (16, 128)) for b in range(2)]
            lhs.append(jnp.where(diag, jnp.concatenate(rows, axis=0), 0.0).astype(BF16))
        lhs = jnp.concatenate(lhs, axis=1)
        arrive(g_q[g])
        for j in range(2):
            q[j] = q[j] + _dot(lhs, w_tile(wq_s, g, j))
    qb = [t.astype(BF16) for t in q]

    idx_c = (lane % 8) * 16 + hl
    qa = [[jnp.zeros((32, 128), F32) for _ in range(4)] for _ in range(2)]
    for g in range(_GW):
        arrive(g_uk[g])
        for j in range(2):
            w = w_tile(wuk_s, g, j)
            for half in range(2):
                sc = _dot_nt(qb[j], w[512 * half:512 * (half + 1)])
                for u in range(4):
                    i, t = tile_pos(4 * half + u, g)
                    picked = jnp.take_along_axis(sc[:, 128 * u:128 * (u + 1)], idx_c, axis=1)
                    qa[j][i] = jnp.where(lane // 8 == t, picked, qa[j][i])
    for j in range(2):
        for i in range(4):
            ob = qa[j][i].astype(BF16)
            for b in range(2):
                qa_s[b, 16 * j:16 * j + 16, 128 * i:128 * (i + 1)] = ob[16 * b:16 * b + 16, :]

    cexp = (_D ** -0.5) * _LOG2E
    ck = _NSK * 32 * _CKG
    for b in range(_B):
        qh = qa_s[b]
        m = jnp.full((32, 1), -jnp.inf, F32)
        l = jnp.zeros((32, 128), F32)
        acc = jnp.zeros((32, _DC), F32)
        for c in range(0, _GK, _CKG):
            for k in range(_CKG):
                arrive(g_kv[b][c + k])
            kv = ckv_s[b, :, c:c + _CKG].reshape(ck, _DC)
            s = _dot_nt(qh, kv)
            m_new = jnp.maximum(m, jnp.max(s, axis=1, keepdims=True))
            alpha = jnp.exp2((m - m_new) * cexp)
            p = jnp.exp2((s - m_new) * cexp)
            ps = p[:, 0:128]
            for u in range(1, ck // 128):
                ps = ps + p[:, 128 * u:128 * (u + 1)]
            l = l * alpha + ps
            acc = acc * alpha + _dot(p.astype(BF16), kv)
            m = m_new
        cc = acc / jnp.sum(l, axis=1, keepdims=True)
        for j in range(2):
            cc_s[j, 16 * b:16 * b + 16, :] = cc[16 * j:16 * j + 16, :]

    ctx = [jnp.zeros((32, 128), F32) for _ in range(2)]
    for g in range(_GW):
        lhs = []
        for j in range(2):
            parts = []
            for s in range(_NSW):
                i, t = tile_pos(s, g)
                z = jnp.take_along_axis(cc_s[j, :, 128 * i:128 * (i + 1)], 8 * t + lane // 16, axis=1)
                parts.append(jnp.where(diag, z, 0.0).astype(BF16))
            lhs.append(jnp.concatenate(parts, axis=1))
        arrive(g_uv[g])
        for j in range(2):
            ctx[j] = ctx[j] + _dot(lhs[j], w_tile(wuv_s, g, j))

    ctx_b = [t.astype(BF16).astype(F32) for t in ctx]
    halves = [[jnp.take_along_axis(ctx_b[j], 64 * dh + lane % 64, axis=1) for dh in range(2)]
              for j in range(2)]
    oacc = jnp.zeros((32, _M), F32)
    for g in range(_GO):
        parts = []
        for k in range(4):
            head = 8 * (k % 2) + 4 * (lane // 64) + g // 2
            parts.append(jnp.where(hl == head, halves[k // 2][g % 2], 0.0).astype(BF16))
        lhs = jnp.concatenate(parts, axis=1)
        arrive(g_o[g])
        oacc = oacc + _dot(lhs, wo_s[:, g].reshape(_NSO * 64, _M))
    o0 = jnp.sum(oacc[0:16], axis=0, keepdims=True)
    o1 = jnp.sum(oacc[16:32], axis=0, keepdims=True)
    r2 = lax.broadcasted_iota(jnp.int32, (2, _M), 0)
    attn = jnp.where(r2 == 0, jnp.broadcast_to(o0, (2, _M)), jnp.broadcast_to(o1, (2, _M)))
    h = x + attn

    hn = _layernorm(h).astype(BF16)
    b1 = b1_s[...].astype(F32).reshape(1, _F)
    out = h
    acts = [None] * nf

    def up(f):
        arrive(g_1[f])
        lo, hi = f_lo[f], f_lo[f] + _F_STEPS[f]
        h1 = _dot(hn, w1_s[:, lo:hi]) + b1[:, lo:hi]
        sp = jnp.log1p(jnp.exp(-jnp.abs(h1))) + jnp.maximum(h1, 0.0)
        acts[f] = (h1 * jnp.tanh(sp)).astype(BF16)

    def down(f, out):
        arrive(g_2[f])
        return out + _dot(acts[f], w2_s[f_lo[f]:f_lo[f] + _F_STEPS[f], :])

    for f in range(nf + _LEAD - 1):
        if f < nf:
            up(f)
        if f >= _LEAD - 1:
            out = down(f - _LEAD + 1, out)
    o_ref[...] = out.astype(o_ref.dtype)


@jax.jit
def pallas_sequential_preLN__compressed_kv_cla__dense_activation_mish__decode_kernel(
    A_x: jax.Array,
    A_c_kv: jax.Array,
    A_w_q: jax.Array,
    A_w_uk: jax.Array,
    A_w_uv: jax.Array,
    A_w_o: jax.Array,
    B_x: jax.Array,
    B_w1: jax.Array,
    B_b1: jax.Array,
    B_w2: jax.Array,
):
    del B_x
    b, sq, m = A_x.shape
    hbm = pl.BlockSpec(memory_space=pl.ANY)
    ckv = A_c_kv.reshape(_B, _NSK, _GK, 32, _DC)
    wq, wuk, wuv = (w.reshape(_NSW, _GW, 8, _H, _D) for w in (A_w_q, A_w_uk, A_w_uv))
    wo = A_w_o.reshape(_NSO, _GO, 64, _M)
    out = pl.pallas_call(
        _kernel,
        out_shape=jax.ShapeDtypeStruct((b * sq, m), A_x.dtype),
        in_specs=[hbm] * 9,
        out_specs=pl.BlockSpec(memory_space=pltpu.VMEM),
        scratch_shapes=[
            pltpu.VMEM(ckv.shape, ckv.dtype),
            pltpu.VMEM(wq.shape, wq.dtype),
            pltpu.VMEM(wuk.shape, wuk.dtype),
            pltpu.VMEM(wuv.shape, wuv.dtype),
            pltpu.VMEM(wo.shape, wo.dtype),
            pltpu.VMEM(B_w1.shape, B_w1.dtype),
            pltpu.VMEM(B_w2.shape, B_w2.dtype),
            pltpu.VMEM((16, 8, 128), F32),
            pltpu.VMEM((_B, _H, _DC), BF16),
            pltpu.VMEM((2, 32, _DC), F32),
            pltpu.VMEM((b * sq, m), A_x.dtype),
            pltpu.VMEM(B_b1.shape, B_b1.dtype),
            pltpu.SemaphoreType.DMA((_RING,)),
        ],
        compiler_params=pltpu.CompilerParams(vmem_limit_bytes=64 * 1024 * 1024),
    )(A_x.reshape(b * sq, m), B_b1, ckv, wq, wuk, wuv, wo, B_w1, B_w2)
    return out.reshape(b, sq, m)
```

```python
import jax
import jax.numpy as jnp
from jax import lax
from jax.experimental import pallas as pl
from jax.experimental.pallas import tpu as pltpu

F32 = jnp.float32
BF16 = jnp.bfloat16

_B, _H, _D, _M, _DC, _SK, _F = 2, 32, 128, 512, 512, 8192, 1792
_EPS = 1e-5
_LOG2E = 1.4426950408889634

_RING = 6
_NS = 8
_GW = 8
_GK = 16
_GO = 8
_G1 = 4
_G2 = 7
_KG = 2


def _layernorm(x):
    m = jnp.mean(x, axis=-1, keepdims=True)
    d = x - m
    v = jnp.mean(d * d, axis=-1, keepdims=True)
    return d * lax.rsqrt(v + _EPS)


def _dot(a, b):
    return jnp.dot(a, b, preferred_element_type=F32)


def _dot_nt(a, b):
    return lax.dot_general(a, b, (((1,), (1,)), ((), ())), preferred_element_type=F32)


def _kernel(x_hbm, b1_hbm, ckv_hbm, wq_hbm, wuk_hbm, wuv_hbm, wo_hbm, w1_hbm, w2_hbm,
            o_ref,
            ckv_s, wq_s, wuk_s, wuv_s, wo_s, w1_s, w2_s, y_s, qa_s, cc_s, x_s, b1_s, sems):
    groups = []

    def add_group(hbm, vmem, lead, g, n_streams, rows, granule):
        copies = [(hbm.at[lead + (s, g, pl.ds(r, granule))],
                   vmem.at[lead + (s, g, pl.ds(r, granule))])
                  for r in range(0, rows, granule) for s in range(n_streams)]
        groups.append((copies, vmem.at[lead + (slice(None), g)]))
        return len(groups) - 1

    groups.append(([(x_hbm, x_s), (b1_hbm, b1_s)], None))
    g_small = 0
    g_q = [add_group(wq_hbm, wq_s, (), g, _NS, 8, 4) for g in range(_GW)]
    g_uk = [add_group(wuk_hbm, wuk_s, (), g, _NS, 8, 4) for g in range(_GW)]
    g_kv = [[add_group(ckv_hbm, ckv_s, (b,), g, _NS, 64, 32) for g in range(_GK)]
            for b in range(_B)]
    g_uv = [add_group(wuv_hbm, wuv_s, (), g, _NS, 8, 4) for g in range(_GW)]
    g_o = [add_group(wo_hbm, wo_s, (), g, _NS, 64, 32) for g in range(_GO)]
    g_1 = [add_group(w1_hbm, w1_s, (), g, _NS, 16, 8) for g in range(_G1)]
    g_2 = [add_group(w2_hbm, w2_s, (), g, 2, 128, 16) for g in range(_G2)]

    def start(g):
        for k, (src, dst) in enumerate(groups[g][0]):
            pltpu.make_async_copy(src, dst, sems.at[g % _RING]).start(priority=k % 2)

    def arrive(g):
        copies, slab = groups[g]
        if slab is None:
            for src, dst in copies:
                pltpu.make_async_copy(src, dst, sems.at[g % _RING]).wait()
        else:
            pltpu.make_async_copy(slab, slab, sems.at[g % _RING]).wait()
        if g + _RING < len(groups):
            start(g + _RING)

    for g in range(_RING):
        start(g)

    row = lax.broadcasted_iota(jnp.int32, (32, 128), 0)
    lane = lax.broadcasted_iota(jnp.int32, (32, 128), 1)
    hl = row % 16
    diag = (lane % 16) == hl

    arrive(g_small)
    x = x_s[...].astype(F32)
    xn = _layernorm(x).astype(BF16).astype(F32)
    for i in range(4):
        y_s[0, 2 * i:2 * i + 2, :] = xn[:, 128 * i:128 * (i + 1)]
    x8 = y_s[0]
    lane8 = lax.broadcasted_iota(jnp.int32, (8, 128), 1)
    for t in range(16):
        y_s[t] = jnp.take_along_axis(x8, 8 * t + lane8 // 16, axis=1)

    def tile_pos(s, g):
        return s // 2, 8 * (s % 2) + g

    def w_tile(ref, g, j):
        return ref[:, g, :, 16 * j:16 * j + 16, :].reshape(_NS * 128, 128)

    q = [jnp.zeros((32, 128), F32) for _ in range(2)]
    for g in range(_GW):
        lhs = []
        for s in range(_NS):
            i, t = tile_pos(s, g)
            rows = [jnp.broadcast_to(y_s[t, 2 * i + b:2 * i + b + 1, :], (16, 128)) for b in range(2)]
            lhs.append(jnp.where(diag, jnp.concatenate(rows, axis=0), 0.0).astype(BF16))
        lhs = jnp.concatenate(lhs, axis=1)
        arrive(g_q[g])
        for j in range(2):
            q[j] = q[j] + _dot(lhs, w_tile(wq_s, g, j))
    qb = [t.astype(BF16) for t in q]

    pick = (lane % 8) * 16 + hl
    qa = [[jnp.zeros((32, 128), F32) for _ in range(4)] for _ in range(2)]
    for g in range(_GW):
        arrive(g_uk[g])
        for j in range(2):
            w = w_tile(wuk_s, g, j)
            for half in range(2):
                sc = _dot_nt(qb[j], w[512 * half:512 * (half + 1)])
                for u in range(4):
                    i, t = tile_pos(4 * half + u, g)
                    picked = jnp.take_along_axis(sc[:, 128 * u:128 * (u + 1)], pick, axis=1)
                    qa[j][i] = jnp.where(lane // 8 == t, picked, qa[j][i])
    for j in range(2):
        for i in range(4):
            ob = qa[j][i].astype(BF16)
            for b in range(_B):
                qa_s[b, 16 * j:16 * j + 16, 128 * i:128 * (i + 1)] = ob[16 * b:16 * b + 16, :]

    cexp = (_D ** -0.5) * _LOG2E
    ck = _NS * 64 * _KG
    for b in range(_B):
        qh = qa_s[b]
        m = jnp.full((32, 1), -jnp.inf, F32)
        l = jnp.zeros((32, 128), F32)
        acc = jnp.zeros((32, _DC), F32)
        for c in range(0, _GK, _KG):
            for k in range(_KG):
                arrive(g_kv[b][c + k])
            kv = ckv_s[b, :, c:c + _KG].reshape(ck, _DC)
            s = _dot_nt(qh, kv)
            m_new = jnp.maximum(m, jnp.max(s, axis=1, keepdims=True))
            alpha = jnp.exp2((m - m_new) * cexp)
            p = jnp.exp2((s - m_new) * cexp)
            ps = p[:, 0:128]
            for u in range(1, ck // 128):
                ps = ps + p[:, 128 * u:128 * (u + 1)]
            l = l * alpha + ps
            acc = acc * alpha + _dot(p.astype(BF16), kv)
            m = m_new
        cc = acc / jnp.sum(l, axis=1, keepdims=True)
        for j in range(2):
            cc_s[j, 16 * b:16 * b + 16, :] = cc[16 * j:16 * j + 16, :]

    ctx = [jnp.zeros((32, 128), F32) for _ in range(2)]
    for g in range(_GW):
        lhs = []
        for j in range(2):
            parts = []
            for s in range(_NS):
                i, t = tile_pos(s, g)
                z = jnp.take_along_axis(cc_s[j, :, 128 * i:128 * (i + 1)], 8 * t + lane // 16, axis=1)
                parts.append(jnp.where(diag, z, 0.0).astype(BF16))
            lhs.append(jnp.concatenate(parts, axis=1))
        arrive(g_uv[g])
        for j in range(2):
            ctx[j] = ctx[j] + _dot(lhs[j], w_tile(wuv_s, g, j))

    ctx_b = [t.astype(BF16).astype(F32) for t in ctx]
    halves = [[jnp.take_along_axis(ctx_b[j], 64 * dh + lane % 64, axis=1) for dh in range(2)]
              for j in range(2)]
    oacc = jnp.zeros((32, _M), F32)
    for g in range(_GO):
        parts = []
        for k in range(4):
            head = 8 * (k % 2) + 4 * (lane // 64) + g // 2
            parts.append(jnp.where(hl == head, halves[k // 2][g % 2], 0.0).astype(BF16))
        lhs = jnp.concatenate(parts, axis=1)
        arrive(g_o[g])
        oacc = oacc + _dot(lhs, wo_s[:, g].reshape(_NS * 64, _M))
    o0 = jnp.sum(oacc[0:16], axis=0, keepdims=True)
    o1 = jnp.sum(oacc[16:32], axis=0, keepdims=True)
    r2 = lax.broadcasted_iota(jnp.int32, (_B, _M), 0)
    attn = jnp.where(r2 == 0, jnp.broadcast_to(o0, (_B, _M)), jnp.broadcast_to(o1, (_B, _M)))
    h = x + attn

    hn = _layernorm(h).astype(BF16)
    b1 = b1_s[...].astype(F32).reshape(1, _F)
    for g in g_1:
        arrive(g)
    h1 = _dot(hn, w1_s[...].reshape(_M, _F)) + b1
    sp = jnp.log1p(jnp.exp(-jnp.abs(h1))) + jnp.maximum(h1, 0.0)
    act = (h1 * jnp.tanh(sp)).astype(BF16)
    out = h
    for f in range(_G2):
        a = jnp.concatenate([act[:, 128 * f:128 * (f + 1)],
                             act[:, _F // 2 + 128 * f:_F // 2 + 128 * (f + 1)]], axis=1)
        arrive(g_2[f])
        out = out + _dot(a, w2_s[:, f].reshape(256, _M))
    o_ref[...] = out.astype(o_ref.dtype)


@jax.jit
def pallas_sequential_preLN__compressed_kv_cla__dense_activation_mish__decode_kernel(
    A_x: jax.Array,
    A_c_kv: jax.Array,
    A_w_q: jax.Array,
    A_w_uk: jax.Array,
    A_w_uv: jax.Array,
    A_w_o: jax.Array,
    B_x: jax.Array,
    B_w1: jax.Array,
    B_b1: jax.Array,
    B_w2: jax.Array,
):
    del B_x
    b, sq, m = A_x.shape
    ckv = A_c_kv.reshape(_B, _NS, _GK, 64, _DC)
    wq, wuk, wuv = (w.reshape(_NS, _GW, 8, _H, _D) for w in (A_w_q, A_w_uk, A_w_uv))
    wo = A_w_o.reshape(_NS, _GO, 64, _M)
    w1 = B_w1.reshape(_NS, _G1, 16, _F)
    w2 = B_w2.reshape(2, _G2, 128, _M)
    big = (ckv, wq, wuk, wuv, wo, w1, w2)
    out = pl.pallas_call(
        _kernel,
        out_shape=jax.ShapeDtypeStruct((b * sq, m), A_x.dtype),
        in_specs=[pl.BlockSpec(memory_space=pl.ANY)] * 9,
        out_specs=pl.BlockSpec(memory_space=pltpu.VMEM),
        scratch_shapes=[pltpu.VMEM(a.shape, a.dtype) for a in big] + [
            pltpu.VMEM((16, 8, 128), F32),
            pltpu.VMEM((_B, _H, _DC), BF16),
            pltpu.VMEM((2, 32, _DC), F32),
            pltpu.VMEM((b * sq, m), A_x.dtype),
            pltpu.VMEM(B_b1.shape, B_b1.dtype),
            pltpu.SemaphoreType.DMA((_RING,)),
        ],
        compiler_params=pltpu.CompilerParams(vmem_limit_bytes=64 * 1024 * 1024),
    )(A_x.reshape(b * sq, m), B_b1, *big)
    return out.reshape(b, sq, m)
```
